```python
import os as _os
_os.environ.setdefault("JAX_PLATFORMS", "cpu")
import jax
import jax.numpy as jnp

def _softmax(x, axis=-1):
    return jax.nn.softmax(x, axis=axis)
def _gelu(x):
    return jax.nn.gelu(x, approximate=True)
def _silu(x):
    return jax.nn.silu(x)
def _sigmoid(x):
    return jax.nn.sigmoid(x)
def _layernorm(x, axis=-1, eps=1e-5):
    m = jnp.mean(x, axis=axis, keepdims=True)
    v = jnp.var(x, axis=axis, keepdims=True)
    return (x - m) / jnp.sqrt(v + eps)
def _scatter_add(tgt, idx, src, axis=0):
    return tgt.at[idx].add(src)
def _segment_sum(src, seg, n):
    return jax.ops.segment_sum(src, seg, n)
class _Rng:
    def __init__(self, key):
        self._k = key
    def _next(self):
        self._k, sub = jax.random.split(self._k)
        return sub
    def normal(self, shape):
        return jax.random.normal(self._next(), shape, dtype=jnp.bfloat16)
    def randint(self, lo, hi, shape):
        return jax.random.randint(self._next(), shape, lo, hi, dtype=jnp.int32)
    def uniform(self, shape, lo=0.0, hi=1.0):
        return jax.random.uniform(self._next(), shape, jnp.bfloat16, lo, hi)
    def permutation(self, n):
        return jax.random.permutation(self._next(), n)


kernel_name = 'sequential_preLN__mha_block__dense_activation_mish__prompt'

def setup_inputs():
    _rng = _Rng(jax.random.key(int.from_bytes(__import__("os").urandom(4), "little")))
    _w = (lambda a: (lambda t: t.astype(jnp.bfloat16) if jnp.issubdtype(t.dtype, jnp.floating) else t)(jnp.asarray(a)))
    def _A_setup():
        B, S, D, H = 1, 2048, 576, 32
        return {
            "x": _w((lambda *s: _rng.normal(s) * 0.05)(B, S, D)),
            "wqkv": _w((lambda *s: _rng.normal(s) * 0.05)(D, 3 * D)),
            "wo": _w((lambda *s: _rng.normal(s) * 0.05)(D, D)),
        }
    _A_in = _A_setup()

    def _B_setup():
        B, S, D, F = 1, 2048, 576, 4608
        return {
            "x": _w((lambda *s: _rng.normal(s) * 0.05)(B, S, D)),
            "w1": _w((lambda *s: _rng.normal(s) * 1.6)(D, F) * (D ** -0.5)),
            "b1": _w((lambda *s: _rng.normal(s) * 0.05)(F)),
            "w2": _w((lambda *s: _rng.normal(s) * 0.05)(F, D) * (F ** -0.5)),
        }
    _B_in = _B_setup()

    return {
        "A_x": _A_in["x"],
        "A_wqkv": _A_in["wqkv"],
        "A_wo": _A_in["wo"],
        "B_x": _B_in["x"],
        "B_w1": _B_in["w1"],
        "B_b1": _B_in["b1"],
        "B_w2": _B_in["w2"],
    }

def reference(A_x, A_wqkv, A_wo, B_x, B_w1, B_b1, B_w2):
    def _A_ref(x, wqkv, wo):
        B, S, D = x.shape
        H = 32
        Dh = D // H
        qkv = (lambda x, *d: x.transpose(*d))((x @ wqkv).reshape(B, S, 3, H, Dh), 2, 0, 3, 1, 4)
        q, k, v = qkv[0], qkv[1], qkv[2]
        scores = jnp.einsum("bhqd,bhkd->bhqk", q, k) * (Dh ** -0.5)
        p = _softmax(scores, axis=-1)
        o = jnp.einsum("bhqk,bhkd->bhqd", p, v)
        return (lambda x, *d: x.transpose(*d))(o, 0, 2, 1, 3).reshape(B, S, D) @ wo

    def _B_ref(x, w1, b1, w2):
        h = jnp.einsum("bsd,df->bsf", x, w1) + b1
        sp = jnp.log1p(jnp.exp(-jnp.abs(h))) + jnp.where(h > 0, h, jnp.zeros_like(h))
        act = h * jnp.tanh(sp)
        return jnp.einsum("bsf,fd->bsd", act, w2)

    x = A_x
    h = x + _A_ref(_layernorm(x, axis=-1), A_wqkv, A_wo)
    h2 = h + _B_ref(_layernorm(h, axis=-1), B_w1, B_b1, B_w2)
    return h2
```

```python
import functools
import math

import jax
import jax.numpy as jnp
from jax.experimental import pallas as pl
from jax.experimental.pallas import tpu as pltpu

_H = 32
_EPS = 1e-5
_HPT = 7

_QB = 512
_KC = 128
_LEAD = 1
_TB1 = 512
_TB3 = 512
_TB = 512
_FC = 512
_FCB = 9

_F32 = jnp.float32
_BF16 = jnp.bfloat16
_NT = (((1,), (1,)), ((), ()))


def _layernorm_t(x):
    m = jnp.mean(x, axis=0, keepdims=True)
    xc = x - m
    v = jnp.mean(xc * xc, axis=0, keepdims=True)
    return xc * jax.lax.rsqrt(v + _EPS)


def _mish(h):
    e = jnp.exp(jnp.minimum(h, 20.0))
    n = e * (e + 2.0)
    return h * n / (n + 2.0)


def _kernel(xt_hbm, wqkv_hbm, wo_hbm, w1_hbm, b1_hbm, w2t_hbm, out_hbm,
            x_v, wqkv_v, wo_v, w1_v, b1_v, w2_v,
            wt_s, wot_s, b1_s, k_s, qt_s, vs_s, ot_s, s0, s1, qm_s,
            hn_s, out_s, in_sem, out_sem, *, S, D, F):
    H = _H
    DH = D // H
    NT7 = -(-H // _HPT)
    LAST = (H - (NT7 - 1) * _HPT) * DH
    LASTP = -(-LAST // 16) * 16
    QROWS = (NT7 - 1) * 128 + LASTP
    QB, KC = _QB, _KC
    NQ, NC = S // QB, S // KC
    NSTEP = H * NQ
    qscale = float(DH ** -0.5 * math.log2(math.e))

    cp_x = pltpu.make_async_copy(xt_hbm, x_v, in_sem.at[0])
    cp_wqkv = pltpu.make_async_copy(wqkv_hbm, wqkv_v, in_sem.at[1])
    cp_wo = pltpu.make_async_copy(wo_hbm, wo_v, in_sem.at[2])
    cp_w1 = pltpu.make_async_copy(w1_hbm, w1_v, in_sem.at[3])
    cp_b1 = pltpu.make_async_copy(b1_hbm, b1_v, in_sem.at[4])
    cp_w2 = pltpu.make_async_copy(w2t_hbm, w2_v, in_sem.at[5])
    for cp in (cp_wqkv, cp_x, cp_wo, cp_b1, cp_w1, cp_w2):
        cp.start()

    cp_wqkv.wait()
    stride = _HPT * DH
    for t in range(NT7):
        rows = 128 if t < NT7 - 1 else LASTP
        wt_s[t * 128:t * 128 + rows, :] = (
            wqkv_v[:, stride * t:stride * t + 128].T)[:rows]
        wt_s[QROWS + t * 128:QROWS + t * 128 + rows, :] = (
            wqkv_v[:, D + stride * t:D + stride * t + 128].T)[:rows]
    for t in range(-(-D // 128)):
        w = min(128, D - t * 128)
        wt_s[2 * QROWS + t * 128:2 * QROWS + t * 128 + w, :] = (
            wqkv_v[:, 2 * D + t * 128:2 * D + t * 128 + w].T)
    qt_s[NT7 - 1, LASTP:, :] = jnp.zeros((128 - LASTP, S), _BF16)
    cp_x.wait()

    TB1 = _TB1
    ones8 = jnp.ones((8, TB1), _F32)

    def qkv_block(c, carry):
        c0 = pl.multiple_of(c * TB1, TB1)
        xn = _layernorm_t(x_v[:, pl.ds(c0, TB1)].astype(_F32)).astype(_BF16)
        qkv = jnp.dot(wt_s[...], xn, preferred_element_type=_F32)
        for t in range(NT7):
            rows = 128 if t < NT7 - 1 else LASTP
            qt_s[t, 0:rows, pl.ds(c0, TB1)] = (
                qkv[t * 128:t * 128 + rows] * qscale).astype(_BF16)
            kt = qkv[QROWS + t * 128:QROWS + t * 128 + rows].astype(_BF16)
            if rows < 128:
                kt = jnp.concatenate([kt, jnp.zeros((128 - rows, TB1), _BF16)], axis=0)
            k_s[t, pl.ds(c0, TB1), :] = kt.T
        for h in range(H):
            a = 2 * QROWS + (DH * h) // 8 * 8
            slab = jnp.concatenate([qkv[a:a + 24], ones8], axis=0)
            vs_s[h, :, pl.ds(c0, TB1)] = slab.astype(_BF16)
        return carry

    jax.lax.fori_loop(0, S // TB1, qkv_block, 0)

    sub32 = jax.lax.broadcasted_iota(jnp.int32, (64, QB), 0)
    row24 = jax.lax.broadcasted_iota(jnp.int32, (24, QB), 0)

    def hq(i):
        h = i // NQ
        return h, i - h * NQ

    def masked_q(i):
        h, qb = hq(i)
        t = h // _HPT
        lo = (h - t * _HPT) * (DH // 2)
        msk = (sub32 >= lo) & (sub32 < lo + DH // 2)
        q = pltpu.bitcast(qt_s[t, :, pl.ds(pl.multiple_of(qb * QB, QB), QB)], jnp.int32)
        return t, pltpu.bitcast(jnp.where(msk, q, 0), _BF16)

    def qk_chunk(t, qm, c, s_ref, mx):
        s = jnp.dot(k_s[t, c * KC:(c + 1) * KC, :], qm, preferred_element_type=_F32)
        s_ref[c * KC:(c + 1) * KC, :] = s
        cm = jnp.max(s.reshape(KC // 8, 8, QB), axis=0)
        return cm if mx is None else jnp.maximum(mx, cm)

    def fin_max(mx):
        return jnp.broadcast_to(jnp.max(mx, axis=0, keepdims=True), (8, QB))

    def pv_chunk(h, c, s_ref, m8, o, z):
        if z is None:
            s = s_ref[c * KC:(c + 1) * KC, :]
        else:
            s = s_ref[pl.ds(pl.multiple_of(z + c * KC, KC), KC), :]
        p = jnp.exp2(s.reshape(KC // 8, 8, QB) - m8[None]).reshape(KC, QB).astype(_BF16)
        r = jnp.dot(vs_s[h, :, c * KC:(c + 1) * KC], p, preferred_element_type=_F32)
        return r if o is None else o + r

    t0, qm0 = masked_q(0)
    mx0 = None
    for c in range(NC):
        mx0 = qk_chunk(t0, qm0, c, s0, mx0)
    m_init = fin_max(mx0)
    qm_s[...] = masked_q(1)[1]

    def att_step(i, s_cur, s_nxt, m8, z, first):
        h, qb = hq(i)
        inx = jnp.minimum(i + 1, NSTEP - 1)
        if first:
            t = hq(inx)[0] // _HPT
            qm = qm_s[...]
        else:
            t, qm = masked_q(inx)
        mx = None
        o = None
        for c in range(NC + _LEAD):
            if c < NC:
                mx = qk_chunk(t, qm, c, s_nxt, mx)
            if c - _LEAD >= 0:
                o = pv_chunk(h, c - _LEAD, s_cur, m8, o, z)
        inv = 1.0 / o[24:32]
        on = (o[0:24].reshape(3, 8, QB) * inv[None]).reshape(24, QB)
        a = (DH * h) // 8 * 8
        r = DH * h - a
        pltpu.store(
            ot_s.at[pl.ds(pl.multiple_of(a, 8), 24), pl.ds(pl.multiple_of(qb * QB, QB), QB)],
            on, mask=(row24 >= r) & (row24 < r + DH))
        return fin_max(mx)

    def att_head(h, m8):
        z = h >> 24
        for u in range(NQ):
            s_cur, s_nxt = (s0, s1) if u % 2 == 0 else (s1, s0)
            m8 = att_step(h * NQ + u, s_cur, s_nxt, m8, None if u == 0 else z, u == 0)
        qm_s[...] = masked_q(jnp.minimum(h * NQ + NQ + 1, NSTEP - 1))[1]
        return m8

    jax.lax.fori_loop(0, H, att_head, m_init)

    cp_wo.wait()
    wot_s[...] = wo_v[...].T
    TB3 = _TB3
    for j in range(S // TB3):
        cols = slice(j * TB3, (j + 1) * TB3)
        hres = x_v[:, cols].astype(_F32) + jnp.dot(
            wot_s[...], ot_s[:, cols].astype(_BF16), preferred_element_type=_F32)
        ot_s[:, cols] = hres
        hn_s[cols, :] = _layernorm_t(hres).astype(_BF16).T

    for cp in (cp_b1, cp_w1, cp_w2):
        cp.wait()
    b1_s[...] = b1_v[...].astype(_F32)
    TB, FC, FCB = _TB, _FC, _FCB
    NFB = F // (FC * FCB)
    NJ = S // TB

    def out_copy(j):
        c0 = pl.multiple_of(j * TB, TB)
        return pltpu.make_async_copy(out_s.at[:, pl.ds(c0, TB)],
                                     out_hbm.at[:, pl.ds(c0, TB)], out_sem.at[j])

    def ffn_body(i, carry):
        j = i // NFB
        fb = i - j * NFB
        c0 = pl.multiple_of(j * TB, TB)
        hn = hn_s[pl.ds(c0, TB), :]
        acc = ot_s[:, pl.ds(c0, TB)]
        for c in range(FCB):
            f0 = pl.multiple_of((fb * FCB + c) * FC, FC)
            r0 = (fb * FCB + c) * (FC // 128)
            hid = jnp.dot(hn, w1_v[:, pl.ds(f0, FC)], preferred_element_type=_F32)
            bias = jnp.concatenate(
                [b1_s[pl.ds(r0 + r, 1), :] for r in range(FC // 128)], axis=1)
            act = _mish(hid + bias).astype(_BF16)
            acc = acc + jax.lax.dot_general(w2_v[:, pl.ds(f0, FC)], act, _NT,
                                            preferred_element_type=_F32)
        if NFB == 1:
            out_s[:, pl.ds(c0, TB)] = acc.astype(_BF16)
            out_copy(j).start()
        else:
            ot_s[:, pl.ds(c0, TB)] = acc

            @pl.when(fb == NFB - 1)
            def _():
                out_s[:, pl.ds(c0, TB)] = ot_s[:, pl.ds(c0, TB)].astype(_BF16)
                out_copy(j).start()
        return carry

    jax.lax.fori_loop(0, NJ * NFB, ffn_body, 0)
    for j in range(NJ):
        out_copy(j).wait()


@jax.jit
def pallas_sequential_preLN__mha_block__dense_activation_mish__prompt_kernel(
    A_x: jax.Array,
    A_wqkv: jax.Array,
    A_wo: jax.Array,
    B_x: jax.Array,
    B_w1: jax.Array,
    B_b1: jax.Array,
    B_w2: jax.Array,
):
    del B_x
    B, S, D = A_x.shape
    F = B_w1.shape[1]
    assert B == 1
    H = _H
    DH = D // H
    NT7 = -(-H // _HPT)
    LAST = (H - (NT7 - 1) * _HPT) * DH
    QROWS = (NT7 - 1) * 128 + -(-LAST // 16) * 16
    hbm = pl.BlockSpec(memory_space=pltpu.MemorySpace.HBM)
    scratch = [
        pltpu.VMEM((D, S), _BF16),
        pltpu.VMEM((D, 3 * D), _BF16),
        pltpu.VMEM((D, D), _BF16),
        pltpu.VMEM((D, F), _BF16),
        pltpu.VMEM((F // 128, 128), _BF16),
        pltpu.VMEM((D, F), _BF16),
        pltpu.VMEM((2 * QROWS + D, D), _BF16),
        pltpu.VMEM((D, D), _BF16),
        pltpu.VMEM((F // 128, 128), _F32),
        pltpu.VMEM((NT7, S, 128), _BF16),
        pltpu.VMEM((NT7, 128, S), _BF16),
        pltpu.VMEM((H, 32, S), _BF16),
        pltpu.VMEM((D, S), _F32),
        pltpu.VMEM((S, _QB), _F32),
        pltpu.VMEM((S, _QB), _F32),
        pltpu.VMEM((128, _QB), _BF16),
        pltpu.VMEM((S, D), _BF16),
        pltpu.VMEM((D, S), _BF16),
        pltpu.SemaphoreType.DMA((6,)),
        pltpu.SemaphoreType.DMA((S // _TB,)),
    ]
    ops = (
        jnp.swapaxes(A_x[0], 0, 1),
        A_wqkv, A_wo, B_w1,
        B_b1.reshape(F // 128, 128),
        jnp.swapaxes(B_w2, 0, 1),
    )
    ops = tuple(pltpu.with_memory_space_constraint(a, pltpu.MemorySpace.HBM) for a in ops)
    out_t = pl.pallas_call(
        functools.partial(_kernel, S=S, D=D, F=F),
        out_shape=jax.ShapeDtypeStruct((D, S), A_x.dtype),
        in_specs=[hbm] * 6,
        out_specs=hbm,
        scratch_shapes=scratch,
        compiler_params=pltpu.CompilerParams(vmem_limit_bytes=110 * 1024 * 1024),
        name="preln_mha_mish_ffn",
    )(*ops)
    return jnp.swapaxes(out_t, 0, 1)[None]
```

```python
import functools
import math

import jax
import jax.numpy as jnp
from jax.experimental import pallas as pl
from jax.experimental.pallas import tpu as pltpu

_H = 32
_EPS = 1e-5
_HPT = 7

_QB = 512
_KC = 128
_UH = 2
_TB1 = 512
_TB3 = 256
_TB = 256

_F32 = jnp.float32
_BF16 = jnp.bfloat16
_NT = (((1,), (1,)), ((), ()))


def _reciprocal(d):
    r = pltpu.reciprocal(d, approx=True)
    return r * (2.0 - d * r)


def _layernorm_t(x):
    m = jnp.mean(x, axis=0, keepdims=True)
    xc = x - m
    v = jnp.mean(xc * xc, axis=0, keepdims=True)
    return xc * jax.lax.rsqrt(v + _EPS)


def _mish(h):
    e = jnp.exp(jnp.minimum(h, 20.0))
    n = e * (e + 2.0)
    return (h * n) * _reciprocal(n + 2.0)


def _pack(x):
    return pltpu.bitcast(x, jnp.int32)


def _unpack(x):
    return pltpu.bitcast(x, _BF16)


def _dims(D):
    DH = D // _H
    nt7 = -(-_H // _HPT)
    last = -(-((_H - (nt7 - 1) * _HPT) * DH) // 16) * 16
    return DH, nt7, last, (nt7 - 1) * 128 + last


def _kernel(xt_hbm, wqkv_hbm, wo_hbm, w1_hbm, b1_hbm, w2t_hbm, out_hbm,
            x_v, wqkv_v, wo_v, w1_v, b1_v, w2_v,
            wt_s, wot_s, b1_s, k_s, qt_s, vs_s, ot_s, s0, s1, qm_s,
            hn_s, out_s, in_sem, out_sem, *, S, D, F):
    H = _H
    DH, NT7, LASTP, QROWS = _dims(D)
    QB, KC = _QB, _KC
    NQ, NC = S // QB, S // KC
    NSTEP = H * NQ
    qscale = float(DH ** -0.5 * math.log2(math.e))

    TB1 = _TB1
    NB1 = S // TB1
    stride = _HPT * DH
    c_q1 = -(-(stride * (NT7 - 1) + 128) // 128) * 128
    c_k1 = -(-(D + stride * (NT7 - 1) + 128) // 128) * 128
    w_parts = [(0, c_q1), (c_q1, c_k1), (c_k1, 3 * D)]
    cp_w = [pltpu.make_async_copy(wqkv_hbm.at[:, pl.ds(a, b - a)], wqkv_v.at[:, pl.ds(a, b - a)],
                                  in_sem.at[i]) for i, (a, b) in enumerate(w_parts)]
    cp_x = [pltpu.make_async_copy(xt_hbm.at[:, pl.ds(c * TB1, TB1)], x_v.at[:, pl.ds(c * TB1, TB1)],
                                  in_sem.at[3 + c]) for c in range(NB1)]
    cp_wo = pltpu.make_async_copy(wo_hbm, wo_v, in_sem.at[3 + NB1])
    cp_b1 = pltpu.make_async_copy(b1_hbm, b1_v, in_sem.at[4 + NB1])
    cp_w1 = pltpu.make_async_copy(w1_hbm, w1_v, in_sem.at[5 + NB1])
    cp_w2 = pltpu.make_async_copy(w2t_hbm, w2_v, in_sem.at[6 + NB1])
    for cp in cp_w + cp_x + [cp_wo, cp_b1, cp_w1, cp_w2]:
        cp.start()

    def store_rows(ref, r0, val):
        ref[r0 // 2:(r0 + val.shape[0]) // 2, :] = _pack(val)

    qt_s[NT7 - 1, LASTP // 2:, :] = jnp.zeros(((128 - LASTP) // 2, S), jnp.int32)
    s1[...] = jnp.zeros(s1.shape, _F32)
    cp_w[0].wait()
    for t in range(NT7):
        rows = 128 if t < NT7 - 1 else LASTP
        store_rows(wt_s, t * 128, (wqkv_v[:, stride * t:stride * t + 128].T)[:rows])
    cp_w[1].wait()
    for t in range(NT7):
        rows = 128 if t < NT7 - 1 else LASTP
        store_rows(wt_s, QROWS + t * 128,
                   (wqkv_v[:, D + stride * t:D + stride * t + 128].T)[:rows])
    cp_w[2].wait()
    for t in range(-(-D // 128)):
        w = min(128, D - t * 128)
        store_rows(wt_s, 2 * QROWS + t * 128,
                   wqkv_v[:, 2 * D + t * 128:2 * D + t * 128 + w].T)
    cp_x[0].wait()

    row24b = jax.lax.broadcasted_iota(jnp.int32, (24, TB1), 0)

    def qkv_block(c, carry):
        c0 = pl.multiple_of(c * TB1, TB1)

        @pl.when(c == 1)
        def _():
            for cc in range(1, NB1):
                cp_x[cc].wait()
        x = x_v[:, pl.ds(c0, TB1)].astype(_F32)
        xc = x - jnp.mean(x, axis=0, keepdims=True)
        rs = jax.lax.rsqrt(jnp.mean(xc * xc, axis=0, keepdims=True) + _EPS)
        qkv = jnp.dot(_unpack(wt_s[...]), xc.astype(_BF16), preferred_element_type=_F32)
        rq = rs * qscale
        for t in range(NT7):
            rows = 128 if t < NT7 - 1 else LASTP
            qq = (qkv[t * 128:t * 128 + rows] * rq).astype(_BF16)
            qt_s[t, 0:rows // 2, pl.ds(c0, TB1)] = _pack(qq)
            kt = (qkv[QROWS + t * 128:QROWS + t * 128 + rows] * rs).astype(_BF16)
            if rows < 128:
                kt = jnp.concatenate([kt, jnp.zeros((128 - rows, TB1), _BF16)], axis=0)
            k_s[t, pl.ds(pl.multiple_of(c0 // 2, TB1 // 2), TB1 // 2), :] = _pack(kt.T)
        vt = (qkv[2 * QROWS:] * rs).astype(_BF16).astype(_F32)
        for h in range(H):
            a = (DH * h) // 8 * 8
            r = DH * h - a
            vs_s[h, :, pl.ds(c0, TB1)] = jnp.where(
                (row24b >= r) & (row24b < r + DH), vt[a:a + 24], 1.0)
        return carry

    jax.lax.fori_loop(0, NB1, qkv_block, 0)
    cp_wo.wait()
    store_rows(wot_s, 0, wo_v[...].T)

    sub32 = jax.lax.broadcasted_iota(jnp.int32, (64, QB), 0)
    row24 = jax.lax.broadcasted_iota(jnp.int32, (24, QB), 0)

    def hq(i):
        h = i // NQ
        return h, i - h * NQ

    def masked_q(i):
        h, qb = hq(i)
        t = h // _HPT
        lo = (h - t * _HPT) * (DH // 2)
        msk = (sub32 >= lo) & (sub32 < lo + DH // 2)
        q = qt_s[t, :, pl.ds(pl.multiple_of(qb * QB, QB), QB)]
        return t, jnp.where(msk, q, 0)

    def qk_chunk(t, qm, c, s_ref, mx):
        kc = _unpack(k_s[t, c * KC // 2:(c + 1) * KC // 2, :])
        s = jnp.dot(kc, qm, preferred_element_type=_F32)
        s_ref[c * KC:(c + 1) * KC, :] = s
        cm = jnp.max(s.reshape(KC // 8, 8, QB), axis=0)
        return cm if mx is None else jnp.maximum(mx, cm)

    def fin_max(mx):
        return jnp.broadcast_to(jnp.max(mx, axis=0, keepdims=True), (8, QB))

    def pv_chunk(h, c, s_ref, m8, o, z):
        if z is None:
            s = s_ref[c * KC:(c + 1) * KC, :]
        else:
            s = s_ref[pl.ds(pl.multiple_of(z + c * KC, KC), KC), :]
        p = jnp.exp2(s.reshape(KC // 8, 8, QB) - m8[None]).reshape(KC, QB).astype(_BF16)
        r = jnp.dot(vs_s[h, :, c * KC:(c + 1) * KC], p, preferred_element_type=_F32)
        return r if o is None else o + r

    def finish(h, qb, o):
        a = (DH * h) // 8 * 8
        r = DH * h - a
        den = jnp.where(r == 0, o[23:24], o[0:1])
        inv = jnp.broadcast_to(_reciprocal(den), (8, QB))
        on = (o.reshape(3, 8, QB) * inv[None]).reshape(24, QB)
        if not isinstance(a, int):
            a = pl.multiple_of(a, 8)
            q0 = pl.multiple_of(qb * QB, QB)
        else:
            q0 = qb * QB
        pltpu.store(ot_s.at[pl.ds(a, 24), pl.ds(q0, QB)], on,
                    mask=(row24 >= r) & (row24 < r + DH))

    qm_s[...] = masked_q(0)[1]

    def att_slot(j, s_cur, s_nxt, mx_cur, z, first, lead):
        h, qb = hq(jnp.maximum(j - 1, 0))
        m8 = fin_max(mx_cur)
        if first:
            t = hq(j)[0] // _HPT
            qm = _unpack(qm_s[...])
        else:
            t, qm = masked_q(j)
            qm = _unpack(qm)
        mx = None
        o = None
        for c in range(NC + lead):
            if c < NC:
                mx = qk_chunk(t, qm, c, s_nxt, mx)
            if c >= lead:
                o = pv_chunk(h, c - lead, s_cur, m8, o, z)
        finish(h, qb, o)
        return mx

    NU = NQ * _UH

    def att_body(hh, mx):
        z = hh >> 24
        for u in range(NU):
            s_cur, s_nxt = (s1, s0) if u % 2 == 0 else (s0, s1)
            mx = att_slot(hh * NU + u, s_cur, s_nxt, mx, None if u == 0 else z, u == 0,
                          0 if u == 0 else 2)
        qm_s[...] = masked_q(jnp.minimum(hh * NU + NU, NSTEP - 1))[1]
        return mx

    mx_last = jax.lax.fori_loop(0, H // _UH, att_body, jnp.zeros((8, QB), _F32))

    def proj(c0, n):
        cols = pl.ds(c0, n)
        ot_s[:, cols] = x_v[:, cols].astype(_F32) + jnp.dot(
            _unpack(wot_s[...]), ot_s[:, cols].astype(_BF16), preferred_element_type=_F32)

    m8 = fin_max(mx_last)
    o = None
    NP3 = (S - QB) // _TB3
    for i in range(NP3):
        proj(i * _TB3, _TB3)
        for c in range(i * NC // NP3, (i + 1) * NC // NP3):
            o = pv_chunk(H - 1, c, s1, m8, o, None)
    finish(H - 1, NQ - 1, o)
    proj(S - QB, QB)

    TB = _TB
    NJ = S // TB

    def out_copy(j):
        c0 = pl.multiple_of(j * TB, TB)
        return pltpu.make_async_copy(out_s.at[:, pl.ds(c0, TB)],
                                     out_hbm.at[:, pl.ds(c0, TB)], out_sem.at[j])

    hn_s[0:TB, :] = _layernorm_t(ot_s[:, 0:TB]).astype(_BF16).T
    for cp in (cp_b1, cp_w1, cp_w2):
        cp.wait()
    b1_s[...] = b1_v[...].astype(_F32)

    def ffn_body(j, carry):
        c0 = pl.multiple_of(j * TB, TB)
        c1 = pl.multiple_of(jnp.minimum(j + 1, NJ - 1) * TB, TB)
        hn = hn_s[pl.ds(c0, TB), :]
        acc = ot_s[:, pl.ds(c0, TB)]
        hid = jnp.dot(hn, w1_v[...], preferred_element_type=_F32)
        hn_s[pl.ds(c1, TB), :] = _layernorm_t(ot_s[:, pl.ds(c1, TB)]).astype(_BF16).T
        bias = jnp.concatenate([b1_s[r:r + 1, :] for r in range(F // 128)], axis=1)
        act = _mish(hid + bias).astype(_BF16)
        acc = acc + jax.lax.dot_general(w2_v[...], act, _NT,
                                        preferred_element_type=_F32)
        out_s[:, pl.ds(c0, TB)] = acc.astype(_BF16)
        out_copy(j).start()
        return carry

    jax.lax.fori_loop(0, NJ, ffn_body, 0)
    for j in range(NJ):
        out_copy(j).wait()


@jax.jit
def pallas_sequential_preLN__mha_block__dense_activation_mish__prompt_kernel(
    A_x: jax.Array,
    A_wqkv: jax.Array,
    A_wo: jax.Array,
    B_x: jax.Array,
    B_w1: jax.Array,
    B_b1: jax.Array,
    B_w2: jax.Array,
):
    del B_x
    B, S, D = A_x.shape
    F = B_w1.shape[1]
    assert B == 1
    H = _H
    _, NT7, _, QROWS = _dims(D)
    hbm = pl.BlockSpec(memory_space=pltpu.MemorySpace.HBM)
    scratch = [
        pltpu.VMEM((D, S), _BF16),
        pltpu.VMEM((D, 3 * D), _BF16),
        pltpu.VMEM((D, D), _BF16),
        pltpu.VMEM((D, F), _BF16),
        pltpu.VMEM((F // 128, 128), _BF16),
        pltpu.VMEM((D, F), _BF16),
        pltpu.VMEM(((2 * QROWS + D) // 2, D), jnp.int32),
        pltpu.VMEM((D // 2, D), jnp.int32),
        pltpu.VMEM((F // 128, 128), _F32),
        pltpu.VMEM((NT7, S // 2, 128), jnp.int32),
        pltpu.VMEM((NT7, 64, S), jnp.int32),
        pltpu.VMEM((H, 24, S), _F32),
        pltpu.VMEM((D, S), _F32),
        pltpu.VMEM((S, _QB), _F32),
        pltpu.VMEM((S, _QB), _F32),
        pltpu.VMEM((64, _QB), jnp.int32),
        pltpu.VMEM((S, D), _BF16),
        pltpu.VMEM((D, S), _BF16),
        pltpu.SemaphoreType.DMA((7 + S // _TB1,)),
        pltpu.SemaphoreType.DMA((S // _TB,)),
    ]
    out_t = pl.pallas_call(
        functools.partial(_kernel, S=S, D=D, F=F),
        out_shape=jax.ShapeDtypeStruct((D, S), A_x.dtype),
        in_specs=[hbm] * 6,
        out_specs=hbm,
        scratch_shapes=scratch,
        compiler_params=pltpu.CompilerParams(vmem_limit_bytes=110 * 1024 * 1024),
        name="preln_mha_mish_ffn",
    )(jnp.swapaxes(A_x[0], 0, 1), A_wqkv, A_wo, B_w1,
      B_b1.reshape(F // 128, 128), jnp.swapaxes(B_w2, 0, 1))
    return jnp.swapaxes(out_t, 0, 1)[None]
```
